```python
import jax
import jax.numpy as jnp

def _softmax(x, axis=-1):
    return jax.nn.softmax(x, axis=axis)
def _gelu(x):
    return jax.nn.gelu(x, approximate=True)
def _silu(x):
    return jax.nn.silu(x)
def _sigmoid(x):
    return jax.nn.sigmoid(x)
def _layernorm(x, axis=-1, eps=1e-5):
    m = jnp.mean(x, axis=axis, keepdims=True)
    v = jnp.var(x, axis=axis, keepdims=True)
    return (x - m) / jnp.sqrt(v + eps)
def _scatter_add(tgt, idx, src, axis=0):
    return tgt.at[idx].add(src)
def _segment_sum(src, seg, n):
    return jax.ops.segment_sum(src, seg, n)
class _Rng:
    def __init__(self, key):
        self._k = key
    def _next(self):
        self._k, sub = jax.random.split(self._k)
        return sub
    def normal(self, shape):
        return jax.random.normal(self._next(), shape, dtype=jnp.bfloat16)
    def randint(self, lo, hi, shape):
        return jax.random.randint(self._next(), shape, lo, hi, dtype=jnp.int32)
    def uniform(self, shape, lo=0.0, hi=1.0):
        return jax.random.uniform(self._next(), shape, jnp.bfloat16, lo, hi)
    def permutation(self, n):
        return jax.random.permutation(self._next(), n)


kernel_name = 'standalone__gqa_block_cached__near_ridge'

def setup_inputs():
    _rng = _Rng(jax.random.key(int.from_bytes(__import__("os").urandom(4), "little")))
    _w = (lambda a: (lambda t: t.astype(jnp.bfloat16) if jnp.issubdtype(t.dtype, jnp.floating) else t)(jnp.asarray(a)))
    B, Sq, D = 16, 240, 640
    Hq, Hkv, Sk, Dh = 32, 32, 1024, 128
    assert Hq % Hkv == 0, (Hq, Hkv)
    return {
        "x": _w((lambda *s: _rng.normal(s) * 0.05)(B, Sq, D)),
        "k_cache": _w((lambda *s: _rng.normal(s) * 0.05)(B, Hkv, Sk, Dh)),
        "v_cache": _w((lambda *s: _rng.normal(s) * 0.05)(B, Hkv, Sk, Dh)),
        "wq": _w((lambda *s: _rng.normal(s) * 0.05)(D, Hq * Dh) * (D ** -0.5)),
        "wo": _w((lambda *s: _rng.normal(s) * 0.05)(Hq * Dh, D) * ((Hq * Dh) ** -0.5)),
    }

def reference(x, k_cache, v_cache, wq, wo):
    B, Sq, D = x.shape
    Hq, Dh = 32, 128
    Hkv = k_cache.shape[1]
    rep = Hq // Hkv
    q = (lambda x, *d: x.transpose(*d))((x @ wq).reshape(B, Sq, Hq, Dh), 0, 2, 1, 3)
    k = jnp.repeat(k_cache, rep, axis=1)
    v = jnp.repeat(v_cache, rep, axis=1)
    scores = jnp.einsum("bhqd,bhkd->bhqk", q, k) * (Dh ** -0.5)
    p = _softmax(scores, axis=-1)
    o = jnp.einsum("bhqk,bhkd->bhqd", p, v)
    return (lambda x, *d: x.transpose(*d))(o, 0, 2, 1, 3).reshape(B, Sq, Hq * Dh) @ wo
```

```python
import jax, jax.numpy as jnp
from jax import lax
import jax.experimental.pallas as pl
import jax.experimental.pallas.tpu as pltpu
G=8
NS=3
NL=1
CH=8
AUTOF=True
SPLITV=True
SCL=False
EARLY=False
ORDER='q01 L q27 K0 q12 K1 D V0 E K2 V1 K3 V2 K4 q78 c4 V3 O03 K5 d4 K6 c5 d5 O35 K7 V6 V7 F57'
RC=16
LOG2E=1.4426950408889634
@jax.jit
def pallas_standalone__gqa_block_cached__near_ridge_kernel(x,k_cache,v_cache,wq,wo):
    B,Sq,D=x.shape; _,H,Sk,Dh=k_cache.shape
    NG=H//G; T=NG*B; GD=G*Dh; DP=D//128
    cs=(Dh**-0.5)*LOG2E
    f32=jnp.float32; bf16=jnp.bfloat16; u32=jnp.uint32
    def kern(x_hbm,k_hbm,v_hbm,wq_hbm,wo_hbm,o_hbm,
             x_buf,wq_buf,wo_buf,kbuf,vbuf,acc,q_scr,p_scr,o_scr,out_buf,
             x_sem,wq_sem,wo_sem,k_sem,v_sem,o_sem):
        def x_cp(b): return pltpu.make_async_copy(x_hbm.at[b],x_buf.at[b],x_sem.at[b])
        def wq_start(j):
            for g in range(G):
                pltpu.make_async_copy(wq_hbm.at[:,pl.ds(pl.multiple_of((j*G+g)*Dh,Dh),Dh)],wq_buf.at[j,g],wq_sem.at[j]).start()
        def wo_start(j):
            for d in range(DP):
                pltpu.make_async_copy(wo_hbm.at[pl.ds(pl.multiple_of(j*GD,GD),GD),pl.ds(d*128,128)],wo_buf.at[j,d],wo_sem.at[j]).start()
        def wq_wait(j): pltpu.make_async_copy(wq_buf.at[j],wq_buf.at[j],wq_sem.at[j]).wait()
        def wo_wait(j): pltpu.make_async_copy(wo_buf.at[j],wo_buf.at[j],wo_sem.at[j]).wait()
        NC=G//CH
        def k_cp(t,s,c):
            j=t//B; b=t%B
            return pltpu.make_async_copy(k_hbm.at[b,pl.ds(j*G+c*CH,CH)],kbuf.at[s,pl.ds(c*CH,CH)],k_sem.at[s*NC+c])
        def v_cp(t,s,c):
            j=t//B; b=t%B
            return pltpu.make_async_copy(v_hbm.at[b,pl.ds(j*G+c*CH,CH)],vbuf.at[s,pl.ds(c*CH,CH)],v_sem.at[s*NC+c])
        def o_cp(b): return pltpu.make_async_copy(out_buf.at[b],o_hbm.at[b],o_sem.at[b])
        ld=lambda v: pltpu.bitcast(v,bf16)
        def qproj(j,b,g0=0,g1=G):
            w=jnp.concatenate([ld(wq_buf.bitcast(u32)[j,g]) for g in range(g0,g1)],axis=1)
            q=(jnp.dot(x_buf[b],w,preferred_element_type=f32)*(1.0 if SCL else cs)).astype(bf16)
            q_scr[:,g0*Dh:g1*Dh]=q
        def oproj(j,g0,g1):
            w=jnp.concatenate([ld(wo_buf.bitcast(u32)[j,d,pl.ds(g0*Dh//2,(g1-g0)*Dh//2),:]) for d in range(DP)],axis=1)
            return jnp.dot(o_scr[:,g0*Dh:g1*Dh],w,preferred_element_type=f32)
        def oproj_last(j,b):
            a=acc[b]+oproj(j,G-NL,G)
            acc[b]=a
            out_buf[b]=a.astype(bf16)
        x_cp(0).start(); wq_start(0)
        k_cp(0,0,0).start(); v_cp(0,0,0).start()
        o_scr[...]=jnp.zeros_like(o_scr)
        x_cp(0).wait(); wq_wait(0)
        for c in range(1,NC):
            k_cp(0,0,c).start(); v_cp(0,0,c).start()
            if c==1: wo_start(0)
        if NC==1: wo_start(0)
        x_cp(1).start()
        for c in range(NC):
            k_cp(1,1,c).start(); v_cp(1,1,c).start()
        k_cp(0,0,0).wait(); v_cp(0,0,0).wait(); wo_wait(0)
        def body(t,s_):
            j=t//B; b=t%B
            tp=jnp.where(t==0,T-1,t-1)
            st={}; a=None
            HK=Sk//2
            def qkh(g,h):
                return lax.dot_general(q_scr[:,g*Dh:(g+1)*Dh],ld(kbuf.bitcast(u32)[s_,g,pl.ds(h*HK//2,HK//2),:]),(((1,),(1,)),((),())),preferred_element_type=f32)
            def soft(g):
                s=jnp.concatenate([st[g,'s0'],st[g,'s1']],axis=1)
                ls=[];ps=[]
                for r in range(0,Sq,RC):
                    sr=s[r:r+RC]
                    m=jnp.max(sr,axis=-1,keepdims=True)
                    p=jnp.exp2((sr-m)*cs) if SCL else jnp.exp2(sr-m)
                    ls.append(jnp.sum(p,axis=-1,keepdims=True))
                    ps.append(p.astype(bf16) if EARLY else p)
                st[g,'p']=jnp.concatenate(ps,axis=0).astype(bf16); st[g,'l']=ls
            def pvh(g,h):
                return jnp.dot(st[g,'p'][:,h*HK:(h+1)*HK],ld(vbuf.bitcast(u32)[s_,g,pl.ds(h*HK//2,HK//2),:]),preferred_element_type=f32)
            def fin(g):
                o=st[g,'o']; ls=st[g,'l']
                for i,r in enumerate(range(0,Sq,RC)):
                    l=ls[i]
                    rc=pl.reciprocal(l,approx=True)
                    rc=rc*(2.0-l*rc)
                    o_scr[r:r+RC,g*Dh:(g+1)*Dh]=(o[r:r+RC]*rc).astype(bf16)
            s1=jnp.where(s_==NS-1,0,s_+1)
            sp=jnp.where(s_==0,NS-1,s_-1)
            for op in ORDER.split():
                kind,n=op[0],op[1:]
                if kind in 'Ka': st[int(n),'s0']=qkh(int(n),0)
                if kind in 'Kb': st[int(n),'s1']=qkh(int(n),1); soft(int(n))
                if kind=='V' and not SPLITV:
                    st[int(n),'o']=jnp.dot(st[int(n),'p'],ld(vbuf.bitcast(u32)[s_,int(n)]),preferred_element_type=f32)
                else:
                    if kind in 'Vc': st[int(n),'o0']=pvh(int(n),0)
                    if kind in 'Vd': st[int(n),'o']=st[int(n),'o0']+pvh(int(n),1)
                if kind=='f' or (kind in 'Vd' and AUTOF): fin(int(n))
                if kind=='W': k_cp(t,s_,int(n)).wait(); v_cp(t,s_,int(n)).wait()
                if kind=='X':
                    @pl.when(b==0)
                    def _(): wo_wait(j)
                if kind=='L': oproj_last(tp//B,tp%B)
                elif kind=='Q': qproj(j,b)
                elif kind=='q': qproj(j,b,int(n[0]),int(n[1]))
                elif kind in 'OF':
                    g0,g1=int(n[0]),int(n[1])
                    if a is None: a=jnp.where(j>0,acc[b],0.0)
                    a=a+oproj(j,g0,g1)
                    if kind=='F': acc[b]=a
                elif kind=='D':
                    @pl.when(t+NS-1<T)
                    def _():
                        for c in range(NC): k_cp(t+NS-1,sp,c).start()
                    @pl.when(t>T-B)
                    def _(): o_cp(b-1).start()
                    @pl.when(t+2<B)
                    def _(): x_cp(t+2).start()
                    @pl.when(jnp.logical_and(b==2,j+1<NG))
                    def _(): wq_start(j+1); wo_start(j+1)
                elif kind=='E':
                    @pl.when(t+NS-1<T)
                    def _():
                        for c in range(NC): v_cp(t+NS-1,sp,c).start()
            @pl.when(t+1<B)
            def _(): x_cp(t+1).wait()
            @pl.when(jnp.logical_and(b==B-1,j+1<NG))
            def _(): wq_wait(j+1); wo_wait(j+1)
            @pl.when(t+1<T)
            def _():
                k_cp(t+1,s1,0).wait(); v_cp(t+1,s1,0).wait()
            return s1
        lax.fori_loop(0,T,body,0)
        oproj_last(NG-1,B-1)
        o_cp(B-1).start()
        for b in range(B): o_cp(b).wait()
    any_=pl.BlockSpec(memory_space=pl.ANY)
    return pl.pallas_call(kern,
        in_specs=[any_]*5,out_specs=any_,
        out_shape=jax.ShapeDtypeStruct((B,Sq,D),x.dtype),
        scratch_shapes=[pltpu.VMEM((B,Sq,D),bf16),pltpu.VMEM((NG,G,D,Dh),bf16),pltpu.VMEM((NG,DP,GD,128),bf16),
                        pltpu.VMEM((NS,G,Sk,Dh),bf16),pltpu.VMEM((NS,G,Sk,Dh),bf16),
                        pltpu.VMEM((B,Sq,D),f32),pltpu.VMEM((Sq,GD),bf16),pltpu.VMEM((2,Sq,Sk),bf16),pltpu.VMEM((Sq,GD),bf16),pltpu.VMEM((B,Sq,D),bf16),
                        pltpu.SemaphoreType.DMA((B,)),pltpu.SemaphoreType.DMA((NG,)),pltpu.SemaphoreType.DMA((NG,)),
                        pltpu.SemaphoreType.DMA((NS*G//CH,)),pltpu.SemaphoreType.DMA((NS*G//CH,)),pltpu.SemaphoreType.DMA((B,))],
        compiler_params=pltpu.CompilerParams(disable_bounds_checks=True,vmem_limit_bytes=100*1024*1024),
    )(x,k_cache,v_cache,wq,wo)
```

```python
import jax, jax.numpy as jnp
from jax import lax
import jax.experimental.pallas as pl
import jax.experimental.pallas.tpu as pltpu
G=8
NS=3
NL=1
CH=2
WOPOS=3
NP=2
KS=4
VS=5
PD=2
ORDER0='N Q L P X F07'
AUTOF=True
SPLITV=True
SCL=False
EARLY=False
ORDER='q01 L q27 K0 q12 K1 D V0 E K2 V1 K3 V2 K4 q78 c4 V3 O03 K5 d4 K6 c5 d5 O35 K7 V6 V7 F57'
RC=16
LOG2E=1.4426950408889634
@jax.jit
def pallas_standalone__gqa_block_cached__near_ridge_kernel(x,k_cache,v_cache,wq,wo):
    B,Sq,D=x.shape; _,H,Sk,Dh=k_cache.shape
    NG=H//G; T=NG*B; GD=G*Dh; DP=D//128
    cs=(Dh**-0.5)*LOG2E
    f32=jnp.float32; bf16=jnp.bfloat16; u32=jnp.uint32
    def kern(x_hbm,k_hbm,v_hbm,wq_hbm,wo_hbm,o_hbm,
             x_buf,wq_buf,wo_buf,kbuf,vbuf,acc,q_scr,p_scr,o_scr,out_buf,
             x_sem,wq_sem,wo_sem,k_sem,v_sem,kc_sem,vc_sem,wqc_sem,woc_sem,o_sem):
        def x_cp(b): return pltpu.make_async_copy(x_hbm.at[b],x_buf.at[b],x_sem.at[b])
        def wq_start(j):
            for g in range(G):
                pltpu.make_async_copy(wq_hbm.at[:,pl.ds(pl.multiple_of((j*G+g)*Dh,Dh),Dh)],wq_buf.at[j,g],wq_sem.at[j]).start()
        def wo_start(j):
            for d in range(DP):
                pltpu.make_async_copy(wo_hbm.at[pl.ds(pl.multiple_of(j*GD,GD),GD),pl.ds(d*128,128)],wo_buf.at[j,d],wo_sem.at[j]).start()
        def wq_wait(j): pltpu.make_async_copy(wq_buf.at[j],wq_buf.at[j],wq_sem.at[j]).wait()
        def wo_wait(j): pltpu.make_async_copy(wo_buf.at[j],wo_buf.at[j],wo_sem.at[j]).wait()
        NC=G//CH
        def k_cp(t,s):
            j=t//B; b=t%B
            return pltpu.make_async_copy(k_hbm.at[b,pl.ds(j*G,G)],kbuf.at[s],k_sem.at[s])
        def v_cp(t,s):
            j=t//B; b=t%B
            return pltpu.make_async_copy(v_hbm.at[b,pl.ds(j*G,G)],vbuf.at[s],v_sem.at[s])
        def kc_cp(t,c): return pltpu.make_async_copy(k_hbm.at[t,pl.ds(c*CH,CH)],kbuf.at[t,pl.ds(c*CH,CH)],kc_sem.at[t*NC+c])
        def vc_cp(t,c): return pltpu.make_async_copy(v_hbm.at[t,pl.ds(c*CH,CH)],vbuf.at[t,pl.ds(c*CH,CH)],vc_sem.at[t*NC+c])
        def o_cp(b): return pltpu.make_async_copy(out_buf.at[b],o_hbm.at[b],o_sem.at[b])
        col=lambda g: pl.ds(g*Dh,Dh) if isinstance(g,int) else pl.ds(pl.multiple_of(g*Dh,Dh),Dh)
        ld=lambda v: pltpu.bitcast(v,bf16)
        def qproj(j,b,g0=0,g1=G):
            w=jnp.concatenate([ld(wq_buf.bitcast(u32)[j,g]) for g in range(g0,g1)],axis=1)
            q=(jnp.dot(x_buf[b],w,preferred_element_type=f32)*(1.0 if SCL else cs)).astype(bf16)
            q_scr[:,g0*Dh:g1*Dh]=q
        def oproj(j,g0,g1):
            w=jnp.concatenate([ld(wo_buf.bitcast(u32)[j,d,pl.ds(g0*Dh//2,(g1-g0)*Dh//2),:]) for d in range(DP)],axis=1)
            return jnp.dot(o_scr[:,g0*Dh:g1*Dh],w,preferred_element_type=f32)
        def oproj_last(j,b):
            a=acc[b]+oproj(j,G-NL,G)
            acc[b]=a
            out_buf[b]=a.astype(bf16)
        def chunk_start(u):
            t=u//NC; c=u%NC
            if not isinstance(u,int):
                @pl.when(c==0)
                def _(): x_cp(t).start()
            elif c==0: x_cp(t).start()
            def wq_():
                for i in range(CH):
                    g=c*CH+i
                    pltpu.make_async_copy(wq_hbm.at[:,col(g)],wq_buf.at[0,g],wqc_sem.at[c]).start()
            def wo_():
                rows=pl.ds(c*CH*Dh if isinstance(c,int) else pl.multiple_of(c*CH*Dh,CH*Dh),CH*Dh)
                for d in range(DP):
                    pltpu.make_async_copy(wo_hbm.at[rows,d*128:(d+1)*128],wo_buf.at[0,d,rows],woc_sem.at[c]).start()
            if isinstance(u,int): wq_()
            else: pl.when(t==0)(wq_)
            kc_cp(t,c).start(); vc_cp(t,c).start()
            if isinstance(u,int): wo_()
            else: pl.when(t==0)(wo_)
        for u in range(PD): chunk_start(u)
        def kv_start(t,s): x_cp(t).start(); k_cp(t,s).start(); v_cp(t,s).start()
        def slow(u,_):
            t=u//NC; c=u%NC
            @pl.when(c==0)
            def _(): x_cp(t).wait()
            @pl.when(t==0)
            def _():
                r=wq_buf.at[0,pl.ds(c*CH,CH)]
                pltpu.make_async_copy(r,r,wqc_sem.at[c]).wait()
                r=wo_buf.at[0,:,pl.ds(c*CH*Dh,CH*Dh)]
                pltpu.make_async_copy(r,r,woc_sem.at[c]).wait()
            kc_cp(t,c).wait(); vc_cp(t,c).wait()
            @pl.when(u+PD<NP*NC)
            def _(): chunk_start(u+PD)
            @pl.when(u==KS)
            def _(): x_cp(NP).start(); k_cp(NP,NP%NS).start()
            @pl.when(u==VS)
            def _(): v_cp(NP,NP%NS).start()
            w=jnp.concatenate([ld(wq_buf.bitcast(u32)[0,c*CH+i]) for i in range(CH)],axis=1)
            q=(jnp.dot(x_buf[t],w,preferred_element_type=f32)*cs).astype(bf16)
            ps=[];os_=[]
            for i in range(CH):
                s=lax.dot_general(q[:,i*Dh:(i+1)*Dh],ld(kbuf.bitcast(u32)[t,c*CH+i]),(((1,),(1,)),((),())),preferred_element_type=f32)
                p=jnp.exp2(s-jnp.max(s,axis=-1,keepdims=True))
                ps.append((p.astype(bf16),jnp.sum(p,axis=-1,keepdims=True)))
            for i in range(CH):
                p,l=ps[i]
                o=jnp.dot(p,ld(vbuf.bitcast(u32)[t,c*CH+i]),preferred_element_type=f32)
                rc=pl.reciprocal(l,approx=True)
                rc=rc*(2.0-l*rc)
                os_.append((o*rc).astype(bf16))
            w=jnp.concatenate([ld(wo_buf.bitcast(u32)[0,d,pl.ds(pl.multiple_of(c*CH*Dh//2,CH*Dh//2),CH*Dh//2),:]) for d in range(DP)],axis=1)
            acc[t]=jnp.where(c>0,acc[t],0.0)+jnp.dot(jnp.concatenate(os_,axis=1),w,preferred_element_type=f32)
        o_scr[...]=jnp.zeros_like(o_scr)
        lax.fori_loop(0,NP*NC,slow,None)
        x_cp(NP).wait(); k_cp(NP,NP%NS).wait(); v_cp(NP,NP%NS).wait()
        kv_start(NP+1,(NP+1)%NS)
        def body(t,s_,order,first):
            j=t//B; b=t%B
            tp=jnp.where(t==0,T-1,t-1)
            st={}; a=None
            HK=Sk//2
            def qkh(g,h):
                return lax.dot_general(q_scr[:,col(g)],ld(kbuf.bitcast(u32)[s_,g,pl.ds(h*HK//2,HK//2),:]),(((1,),(1,)),((),())),preferred_element_type=f32)
            def soft(g):
                s=jnp.concatenate([st[g,'s0'],st[g,'s1']],axis=1)
                ls=[];ps=[]
                for r in range(0,Sq,RC):
                    sr=s[r:r+RC]
                    m=jnp.max(sr,axis=-1,keepdims=True)
                    p=jnp.exp2((sr-m)*cs) if SCL else jnp.exp2(sr-m)
                    ls.append(jnp.sum(p,axis=-1,keepdims=True))
                    ps.append(p.astype(bf16) if EARLY else p)
                st[g,'p']=jnp.concatenate(ps,axis=0).astype(bf16); st[g,'l']=ls
            def pvh(g,h,u=None):
                return jnp.dot(st[g if u is None else u,'p'][:,h*HK:(h+1)*HK],ld(vbuf.bitcast(u32)[s_,g,pl.ds(h*HK//2,HK//2),:]),preferred_element_type=f32)
            def fin(g,gg=None):
                o=st[g,'o']; ls=st[g,'l']
                if gg is not None: g=gg
                for i,r in enumerate(range(0,Sq,RC)):
                    l=ls[i]
                    rc=pl.reciprocal(l,approx=True)
                    rc=rc*(2.0-l*rc)
                    o_scr[r:r+RC,col(g)]=(o[r:r+RC]*rc).astype(bf16)
            s1=jnp.where(s_==NS-1,0,s_+1)
            sp=jnp.where(s_==0,NS-1,s_-1)
            for op in order.split():
                kind,n=op[0],op[1:]
                if kind in 'Ka': st[int(n),'s0']=qkh(int(n),0)
                if kind in 'Kb': st[int(n),'s1']=qkh(int(n),1); soft(int(n))
                if kind=='V' and not SPLITV:
                    st[int(n),'o']=jnp.dot(st[int(n),'p'],ld(vbuf.bitcast(u32)[s_,int(n)]),preferred_element_type=f32)
                else:
                    if kind in 'Vc': st[int(n),'o0']=pvh(int(n),0)
                    if kind in 'Vd': st[int(n),'o']=st[int(n),'o0']+pvh(int(n),1)
                if kind=='f' or (kind in 'Vd' and AUTOF): fin(int(n))
                if kind=='P':
                    def pair(pi,_):
                        kc_cp(t,pi).wait(); vc_cp(t,pi).wait()
                        for u in range(CH):
                            st[u,'s0']=qkh(pi*CH+u,0); st[u,'s1']=qkh(pi*CH+u,1); soft(u)
                        for u in range(CH):
                            st[u,'o']=pvh(pi*CH+u,0,u)+pvh(pi*CH+u,1,u); fin(u,pi*CH+u)
                    lax.fori_loop(0,NC,pair,None)
                if kind=='N':
                    @pl.when(t+2>2)
                    def _():
                        x_cp(t+2).start(); k_cp(t+2,sp).start(); v_cp(t+2,sp).start()
                if kind=='W': kc_cp(t,int(n)).wait(); vc_cp(t,int(n)).wait()
                if kind=='X':
                    @pl.when(t==0)
                    def _(): wo_wait(0)
                if kind=='L': oproj_last(tp//B,tp%B)
                elif kind=='Q': qproj(j,b)
                elif kind=='q': qproj(j,b,int(n[0]),int(n[1]))
                elif kind in 'OF':
                    g0,g1=int(n[0]),int(n[1])
                    if a is None: a=jnp.where(j>0,acc[b],0.0)
                    a=a+oproj(j,g0,g1)
                    if kind=='F': acc[b]=a
                elif kind=='D':
                    @pl.when(t+NS-1<T)
                    def _(): k_cp(t+NS-1,sp).start()
                    @pl.when(t>T-B)
                    def _(): o_cp(b-1).start()
                    @pl.when(t+2<B)
                    def _(): x_cp(t+2).start()
                    @pl.when(jnp.logical_and(b==4,j+1<NG))
                    def _(): wq_start(j+1); wo_start(j+1)
                elif kind=='E':
                    @pl.when(t+NS-1<T)
                    def _(): v_cp(t+NS-1,sp).start()
            @pl.when(t+1<B)
            def _(): x_cp(t+1).wait()
            @pl.when(jnp.logical_and(b==B-1,j+1<NG))
            def _(): wq_wait(j+1); wo_wait(j+1)
            @pl.when(t==NP-1 if first else t+1<T)
            def _():
                k_cp(t+1,s1).wait(); v_cp(t+1,s1).wait()
            return s1
        lax.fori_loop(NP,T,lambda t,s_:body(t,s_,ORDER,False),NP%NS)
        oproj_last(NG-1,B-1)
        o_cp(B-1).start()
        for b in range(B): o_cp(b).wait()
    any_=pl.BlockSpec(memory_space=pl.ANY)
    return pl.pallas_call(kern,
        in_specs=[any_]*5,out_specs=any_,
        out_shape=jax.ShapeDtypeStruct((B,Sq,D),x.dtype),
        scratch_shapes=[pltpu.VMEM((B,Sq,D),bf16),pltpu.VMEM((NG,G,D,Dh),bf16),pltpu.VMEM((NG,DP,GD,128),bf16),
                        pltpu.VMEM((NS,G,Sk,Dh),bf16),pltpu.VMEM((NS,G,Sk,Dh),bf16),
                        pltpu.VMEM((B,Sq,D),f32),pltpu.VMEM((Sq,GD),bf16),pltpu.VMEM((2,Sq,Sk),bf16),pltpu.VMEM((Sq,GD),bf16),pltpu.VMEM((B,Sq,D),bf16),
                        pltpu.SemaphoreType.DMA((B,)),pltpu.SemaphoreType.DMA((NG,)),pltpu.SemaphoreType.DMA((NG,)),
                        pltpu.SemaphoreType.DMA((NS,)),pltpu.SemaphoreType.DMA((NS,)),pltpu.SemaphoreType.DMA((NP*G//CH,)),pltpu.SemaphoreType.DMA((NP*G//CH,)),pltpu.SemaphoreType.DMA((G//CH,)),pltpu.SemaphoreType.DMA((G//CH,)),pltpu.SemaphoreType.DMA((B,))],
        compiler_params=pltpu.CompilerParams(disable_bounds_checks=True,vmem_limit_bytes=100*1024*1024),
    )(x,k_cache,v_cache,wq,wo)
```

```python
import jax
import jax.numpy as jnp
from jax import lax
import jax.experimental.pallas as pl
import jax.experimental.pallas.tpu as pltpu

G = 8
NS = 3
CH = 2
NP = 2
PD = 2
KS, VS = 4, 5
RC = 16
LOG2E = 1.4426950408889634
ORDER = "q01 L q27 K0 q12 K1 E M D V0 K2 V1 K3 V2 K4 q78 V3 O03 K5 V4 K6 V5 O35 K7 V6 V7 F57"


@jax.jit
def pallas_standalone__gqa_block_cached__near_ridge_kernel(x, k_cache, v_cache, wq, wo):
    B, Sq, D = x.shape
    _, H, Sk, Dh = k_cache.shape
    assert wq.shape == (D, H * Dh) and H % G == 0 and D % 128 == 0 and B > 4
    NG = H // G
    T = NG * B
    GD = G * Dh
    DP = D // 128
    NC = G // CH
    HK = Sk // 2
    scale = (Dh ** -0.5) * LOG2E
    f32, bf16, u32 = jnp.float32, jnp.bfloat16, jnp.uint32
    nt_dims = (((1,), (1,)), ((), ()))

    def kern(x_hbm, k_hbm, v_hbm, wq_hbm, wo_hbm, o_hbm,
             x_buf, wq_buf, wo_buf, kbuf, vbuf, acc, q_scr, o_scr, out_buf,
             x_sem, wq_sem, wo_sem, k_sem, v_sem, kc_sem, vc_sem, wqc_sem, woc_sem, o_sem):
        def window(i, n):
            return pl.ds(i * n if isinstance(i, int) else pl.multiple_of(i * n, n), n)

        def ld(packed):
            return pltpu.bitcast(packed, bf16)

        def wait_all(ref, sem):
            pltpu.make_async_copy(ref, ref, sem).wait()

        def x_cp(b):
            return pltpu.make_async_copy(x_hbm.at[b], x_buf.at[b], x_sem.at[b])

        def k_cp(t, s):
            return pltpu.make_async_copy(k_hbm.at[t % B, pl.ds((t // B) * G, G)], kbuf.at[s], k_sem.at[s])

        def v_cp(t, s):
            return pltpu.make_async_copy(v_hbm.at[t % B, pl.ds((t // B) * G, G)], vbuf.at[s], v_sem.at[s])

        def kc_cp(t, c):
            return pltpu.make_async_copy(
                k_hbm.at[t, pl.ds(c * CH, CH)], kbuf.at[t, pl.ds(c * CH, CH)], kc_sem.at[t * NC + c])

        def vc_cp(t, c):
            return pltpu.make_async_copy(
                v_hbm.at[t, pl.ds(c * CH, CH)], vbuf.at[t, pl.ds(c * CH, CH)], vc_sem.at[t * NC + c])

        def o_cp(b):
            return pltpu.make_async_copy(out_buf.at[b], o_hbm.at[b], o_sem.at[b])

        def w_start(j):
            for g in range(G):
                pltpu.make_async_copy(wq_hbm.at[:, window(j * G + g, Dh)], wq_buf.at[j, g], wq_sem.at[j]).start()
            for d in range(DP):
                pltpu.make_async_copy(
                    wo_hbm.at[window(j, GD), pl.ds(d * 128, 128)], wo_buf.at[j, d], wo_sem.at[j]).start()

        def recip(l):
            r = pl.reciprocal(l, approx=True)
            return r * (2.0 - l * r)

        def qproj(j, b, g0, g1):
            w = jnp.concatenate([ld(wq_buf.bitcast(u32)[j, g]) for g in range(g0, g1)], axis=1)
            q_scr[:, g0 * Dh:g1 * Dh] = (jnp.dot(x_buf[b], w, preferred_element_type=f32) * scale).astype(bf16)

        def oproj(j, g0, g1):
            w = jnp.concatenate(
                [ld(wo_buf.bitcast(u32)[j, d, pl.ds(g0 * Dh // 2, (g1 - g0) * Dh // 2), :]) for d in range(DP)],
                axis=1)
            return jnp.dot(o_scr[:, g0 * Dh:g1 * Dh], w, preferred_element_type=f32)

        def oproj_last(j, b):
            a = acc[b] + oproj(j, G - 1, G)
            acc[b] = a
            out_buf[b] = a.astype(bf16)

        def chunk_start(u):
            t, c = u // NC, u % NC
            static = isinstance(u, int)

            def start_x():
                x_cp(t).start()

            def start_wq():
                for i in range(CH):
                    g = c * CH + i
                    pltpu.make_async_copy(wq_hbm.at[:, window(g, Dh)], wq_buf.at[0, g], wqc_sem.at[c]).start()

            def start_wo():
                rows = window(c, CH * Dh)
                for d in range(DP):
                    pltpu.make_async_copy(
                        wo_hbm.at[rows, d * 128:(d + 1) * 128], wo_buf.at[0, d, rows], woc_sem.at[c]).start()

            if static:
                assert t == 0
                if c == 0:
                    start_x()
                start_wq()
            else:
                pl.when(c == 0)(start_x)
                pl.when(t == 0)(start_wq)
            kc_cp(t, c).start()
            vc_cp(t, c).start()
            if static:
                start_wo()
            else:
                pl.when(t == 0)(start_wo)

        for u in range(PD):
            chunk_start(u)

        def warm(u, carry):
            t, c = u // NC, u % NC

            @pl.when(c == 0)
            def _():
                x_cp(t).wait()

            @pl.when(t == 0)
            def _():
                wait_all(wq_buf.at[0, pl.ds(c * CH, CH)], wqc_sem.at[c])
                wait_all(wo_buf.at[0, :, pl.ds(c * CH * Dh, CH * Dh)], woc_sem.at[c])

            kc_cp(t, c).wait()
            vc_cp(t, c).wait()

            @pl.when(u + PD < NP * NC)
            def _():
                chunk_start(u + PD)

            @pl.when(u == KS)
            def _():
                x_cp(NP).start()
                k_cp(NP, NP % NS).start()

            @pl.when(u == VS)
            def _():
                v_cp(NP, NP % NS).start()

            w = jnp.concatenate([ld(wq_buf.bitcast(u32)[0, c * CH + i]) for i in range(CH)], axis=1)
            q = (jnp.dot(x_buf[t], w, preferred_element_type=f32) * scale).astype(bf16)
            ps, outs = [], []
            for i in range(CH):
                s = lax.dot_general(q[:, i * Dh:(i + 1) * Dh], ld(kbuf.bitcast(u32)[t, c * CH + i]), nt_dims,
                                    preferred_element_type=f32)
                p = jnp.exp2(s - jnp.max(s, axis=-1, keepdims=True))
                ps.append((p.astype(bf16), jnp.sum(p, axis=-1, keepdims=True)))
            for i in range(CH):
                p, l = ps[i]
                o = jnp.dot(p, ld(vbuf.bitcast(u32)[t, c * CH + i]), preferred_element_type=f32)
                outs.append((o * recip(l)).astype(bf16))
            w = jnp.concatenate(
                [ld(wo_buf.bitcast(u32)[0, d, window(c, CH * Dh // 2), :]) for d in range(DP)], axis=1)
            acc[t] = jnp.where(c > 0, acc[t], 0.0) + jnp.dot(
                jnp.concatenate(outs, axis=1), w, preferred_element_type=f32)
            return carry

        o_scr[...] = jnp.zeros_like(o_scr)
        lax.fori_loop(0, NP * NC, warm, None)
        x_cp(NP).wait()
        k_cp(NP, NP % NS).wait()
        v_cp(NP, NP % NS).wait()
        x_cp(NP + 1).start()
        k_cp(NP + 1, (NP + 1) % NS).start()
        v_cp(NP + 1, (NP + 1) % NS).start()

        def body(t, slot):
            j, b = t // B, t % B
            next_slot = jnp.where(slot == NS - 1, 0, slot + 1)
            free_slot = jnp.where(slot == 0, NS - 1, slot - 1)

            def scores(g):
                q = q_scr[:, g * Dh:(g + 1) * Dh]
                s = jnp.concatenate(
                    [lax.dot_general(q, ld(kbuf.bitcast(u32)[slot, g, pl.ds(h * HK // 2, HK // 2), :]), nt_dims,
                                     preferred_element_type=f32) for h in range(2)], axis=1)
                ps, ls = [], []
                for r in range(0, Sq, RC):
                    sr = s[r:r + RC]
                    p = jnp.exp2(sr - jnp.max(sr, axis=-1, keepdims=True))
                    ls.append(jnp.sum(p, axis=-1, keepdims=True))
                    ps.append(p)
                return jnp.concatenate(ps, axis=0).astype(bf16), ls

            def attend(g, p, ls):
                o0, o1 = [jnp.dot(p[:, h * HK:(h + 1) * HK],
                                  ld(vbuf.bitcast(u32)[slot, g, pl.ds(h * HK // 2, HK // 2), :]),
                                  preferred_element_type=f32) for h in range(2)]
                o = o0 + o1
                for l, r in zip(ls, range(0, Sq, RC)):
                    o_scr[r:r + RC, g * Dh:(g + 1) * Dh] = (o[r:r + RC] * recip(l)).astype(bf16)

            probs, a = {}, None
            for op in ORDER.split():
                kind, n = op[0], [int(ch) for ch in op[1:]]
                if kind == "q":
                    qproj(j, b, *n)
                elif kind == "K":
                    probs[n[0]] = scores(n[0])
                elif kind == "V":
                    attend(n[0], *probs[n[0]])
                elif kind == "L":
                    oproj_last((t - 1) // B, (t - 1) % B)
                elif kind in "OF":
                    if a is None:
                        a = jnp.where(j > 0, acc[b], 0.0)
                    a = a + oproj(j, *n)
                    if kind == "F":
                        acc[b] = a
                elif kind == "D":
                    @pl.when(t + 2 < T)
                    def _():
                        k_cp(t + 2, free_slot).start()
                elif kind == "E":
                    @pl.when(t + 2 < T)
                    def _():
                        v_cp(t + 2, free_slot).start()
                elif kind == "M":
                    @pl.when(t > T - B)
                    def _():
                        o_cp(b - 1).start()

                    @pl.when(t + 2 < B)
                    def _():
                        x_cp(t + 2).start()

                    @pl.when(jnp.logical_and(b == 4, j + 1 < NG))
                    def _():
                        w_start(j + 1)

            @pl.when(t + 1 < B)
            def _():
                x_cp(t + 1).wait()

            @pl.when(jnp.logical_and(b == B - 1, j + 1 < NG))
            def _():
                wait_all(wq_buf.at[j + 1], wq_sem.at[j + 1])
                wait_all(wo_buf.at[j + 1], wo_sem.at[j + 1])

            @pl.when(t + 1 < T)
            def _():
                k_cp(t + 1, next_slot).wait()
                v_cp(t + 1, next_slot).wait()

            return next_slot

        lax.fori_loop(NP, T, body, NP % NS)
        oproj_last(NG - 1, B - 1)
        o_cp(B - 1).start()
        for b in range(B):
            o_cp(b).wait()

    hbm = pl.BlockSpec(memory_space=pl.ANY)
    dma = pltpu.SemaphoreType.DMA
    return pl.pallas_call(
        kern,
        in_specs=[hbm] * 5,
        out_specs=hbm,
        out_shape=jax.ShapeDtypeStruct((B, Sq, D), x.dtype),
        scratch_shapes=[
            pltpu.VMEM((B, Sq, D), bf16),
            pltpu.VMEM((NG, G, D, Dh), bf16),
            pltpu.VMEM((NG, DP, GD, 128), bf16),
            pltpu.VMEM((NS, G, Sk, Dh), bf16),
            pltpu.VMEM((NS, G, Sk, Dh), bf16),
            pltpu.VMEM((B, Sq, D), f32),
            pltpu.VMEM((Sq, GD), bf16),
            pltpu.VMEM((Sq, GD), bf16),
            pltpu.VMEM((B, Sq, D), bf16),
            dma((B,)), dma((NG,)), dma((NG,)), dma((NS,)), dma((NS,)),
            dma((NP * NC,)), dma((NP * NC,)), dma((NC,)), dma((NC,)), dma((B,)),
        ],
        compiler_params=pltpu.CompilerParams(
            disable_bounds_checks=True, vmem_limit_bytes=100 * 1024 * 1024),
    )(x, k_cache, v_cache, wq, wo)
```
